```python
import os as _os
_os.environ.setdefault("JAX_PLATFORMS", "cpu")
import jax
import jax.numpy as jnp

def _softmax(x, axis=-1):
    return jax.nn.softmax(x, axis=axis)
def _gelu(x):
    return jax.nn.gelu(x, approximate=True)
def _silu(x):
    return jax.nn.silu(x)
def _sigmoid(x):
    return jax.nn.sigmoid(x)
def _layernorm(x, axis=-1, eps=1e-5):
    m = jnp.mean(x, axis=axis, keepdims=True)
    v = jnp.var(x, axis=axis, keepdims=True)
    return (x - m) / jnp.sqrt(v + eps)
def _scatter_add(tgt, idx, src, axis=0):
    return tgt.at[idx].add(src)
def _segment_sum(src, seg, n):
    return jax.ops.segment_sum(src, seg, n)
class _Rng:
    def __init__(self, key):
        self._k = key
    def _next(self):
        self._k, sub = jax.random.split(self._k)
        return sub
    def normal(self, shape):
        return jax.random.normal(self._next(), shape, dtype=jnp.bfloat16)
    def randint(self, lo, hi, shape):
        return jax.random.randint(self._next(), shape, lo, hi, dtype=jnp.int32)
    def uniform(self, shape, lo=0.0, hi=1.0):
        return jax.random.uniform(self._next(), shape, jnp.bfloat16, lo, hi)
    def permutation(self, n):
        return jax.random.permutation(self._next(), n)


kernel_name = 'concat_heads__mha_block_cached__mha_block_cached__near_ridge'

def setup_inputs():
    _rng = _Rng(jax.random.key(int.from_bytes(__import__("os").urandom(4), "little")))
    _w = (lambda a: (lambda t: t.astype(jnp.bfloat16) if jnp.issubdtype(t.dtype, jnp.floating) else t)(jnp.asarray(a)))
    def _A_setup():
        B, Sq, D = 32, 32, 640
        H, Sk, Dh = 32, 32, 128
        return {
            "x": _w((lambda *s: _rng.normal(s) * 0.8)(B, Sq, D)),
            "k_cache": _w((lambda *s: _rng.normal(s) * 0.8)(B, H, Sk, Dh)),
            "v_cache": _w((lambda *s: _rng.normal(s) * 0.05)(B, H, Sk, Dh)),
            "wq": _w((lambda *s: _rng.normal(s) * 0.8)(D, H * Dh) * (D ** -0.5)),
            "wo": _w((lambda *s: _rng.normal(s) * 0.05)(H * Dh, D) * ((H * Dh) ** -0.5)),
        }
    _A_in = _A_setup()

    def _B_setup():
        B, Sq, D = 32, 32, 640
        H, Sk, Dh = 32, 32, 128
        return {
            "x": _w((lambda *s: _rng.normal(s) * 0.8)(B, Sq, D)),
            "k_cache": _w((lambda *s: _rng.normal(s) * 0.8)(B, H, Sk, Dh)),
            "v_cache": _w((lambda *s: _rng.normal(s) * 0.05)(B, H, Sk, Dh)),
            "wq": _w((lambda *s: _rng.normal(s) * 0.8)(D, H * Dh) * (D ** -0.5)),
            "wo": _w((lambda *s: _rng.normal(s) * 0.05)(H * Dh, D) * ((H * Dh) ** -0.5)),
        }
    _B_in = _B_setup()

    return {
        "A_x": _A_in["x"],
        "A_k_cache": _A_in["k_cache"],
        "A_v_cache": _A_in["v_cache"],
        "A_wq": _A_in["wq"],
        "A_wo": _A_in["wo"],
        "B_x": _B_in["x"],
        "B_k_cache": _B_in["k_cache"],
        "B_v_cache": _B_in["v_cache"],
        "B_wq": _B_in["wq"],
        "B_wo": _B_in["wo"],
    }

def reference(A_x, A_k_cache, A_v_cache, A_wq, A_wo, B_x, B_k_cache, B_v_cache, B_wq, B_wo):
    def _A_ref(x, k_cache, v_cache, wq, wo):
        B, Sq, D = x.shape
        H, Dh = 32, 128
        q = (lambda x, *d: x.transpose(*d))((x @ wq).reshape(B, Sq, H, Dh), 0, 2, 1, 3)
        scores = jnp.einsum("bhqd,bhkd->bhqk", q, k_cache) * (Dh ** -0.5)
        p = _softmax(scores, axis=-1)
        o = jnp.einsum("bhqk,bhkd->bhqd", p, v_cache)
        return (lambda x, *d: x.transpose(*d))(o, 0, 2, 1, 3).reshape(B, Sq, H * Dh) @ wo

    def _B_ref(x, k_cache, v_cache, wq, wo):
        B, Sq, D = x.shape
        H, Dh = 32, 128
        q = (lambda x, *d: x.transpose(*d))((x @ wq).reshape(B, Sq, H, Dh), 0, 2, 1, 3)
        scores = jnp.einsum("bhqd,bhkd->bhqk", q, k_cache) * (Dh ** -0.5)
        p = _softmax(scores, axis=-1)
        o = jnp.einsum("bhqk,bhkd->bhqd", p, v_cache)
        return (lambda x, *d: x.transpose(*d))(o, 0, 2, 1, 3).reshape(B, Sq, H * Dh) @ wo

    a = _A_ref(A_x, A_k_cache, A_v_cache, A_wq, A_wo)
    b = _B_ref(B_x, B_k_cache, B_v_cache, B_wq, B_wo)
    return jnp.concatenate([a, b], axis=-1)
```

```python
import jax
import jax.numpy as jnp
from jax import lax
import jax.experimental.pallas as pl
import jax.experimental.pallas.tpu as pltpu

B, SQ, D = 32, 32, 640
H, SK, DH = 32, 32, 128
M = B * SQ
HC = 4
NC = H // HC
CW = HC * DH
NG = B // 4
SCALE = DH ** -0.5
F32 = jnp.float32
BF16 = jnp.bfloat16


def _kernel(ax, ak, av, awq, awo, bx, bk, bv, bwq, bwo, out_hbm,
            x_buf, wq_buf, wo_buf, k_buf, v_buf, q_s, o_s, acc, stage,
            sem_x, sem_w, sem_o):
    blocks = ((ax, ak, av, awq, awo), (bx, bk, bv, bwq, bwo))

    def chunk_copies(blk, c, slot):
        _, k, v, wq, wo = blocks[blk]
        return (
            pltpu.make_async_copy(wq.at[:, pl.ds(c * CW, CW)], wq_buf.at[slot], sem_w.at[0, slot]),
            pltpu.make_async_copy(k.at[:, pl.ds(c * HC, HC)], k_buf.at[slot], sem_w.at[1, slot]),
            pltpu.make_async_copy(v.at[:, pl.ds(c * HC, HC)], v_buf.at[slot], sem_w.at[2, slot]),
            pltpu.make_async_copy(wo.at[pl.ds(c * CW, CW), :], wo_buf.at[slot], sem_w.at[3, slot]),
        )

    def x_copy(blk):
        return pltpu.make_async_copy(blocks[blk][0], x_buf.at[blk], sem_x.at[blk])

    def out_copy(blk):
        return pltpu.make_async_copy(stage.at[blk], out_hbm.at[:, pl.ds(blk * D, D)], sem_o.at[blk])

    lane_blk = lax.broadcasted_iota(jnp.int32, (SQ, 128), 1) // SQ

    def st_stage(g, slot):
        r0 = g * 128
        b0 = g * 4
        sts = []
        for h in range(HC):
            q4 = q_s[pl.ds(r0, 128), h * DH:(h + 1) * DH]
            k4 = k_buf[slot, pl.ds(b0, 4), h].reshape(128, DH)
            sts.append(lax.dot_general(k4, q4, (((1,), (1,)), ((), ())), preferred_element_type=F32))
        return sts

    def sm_stage(sts):
        pts = []
        for st in sts:
            t = st[0:SK]
            for j in range(1, 4):
                t = jnp.where(lane_blk == j, st[SK * j:SK * (j + 1)], t)
            m = jnp.max(t, axis=0, keepdims=True)
            e = jnp.exp((t - m) * SCALE)
            l = jnp.sum(e, axis=0, keepdims=True)
            pts.append(e * (1.0 / l))
        pt_all = jnp.concatenate(pts, axis=0)
        return pt_all.T

    def pv_stage(g, slot, p_all):
        r0 = g * 128
        b0 = g * 4
        for b in range(4):
            pb = p_all[SQ * b:SQ * (b + 1)]
            p_bd = jnp.concatenate(
                [jnp.where(lane_blk == h, pb, 0.0) for h in range(HC)], axis=0).astype(BF16)
            v4 = v_buf[slot, b0 + b].reshape(128, DH)
            ob = jnp.dot(p_bd, v4, preferred_element_type=F32)
            for h in range(HC):
                o_s[pl.ds(r0 + SQ * b, SQ), h * DH:(h + 1) * DH] = ob[SQ * h:SQ * (h + 1)].astype(BF16)

    def attention(slot):
        ps = [None] * NG
        sts = st_stage(0, slot)
        for g in range(NG + 1):
            nxt = st_stage(g + 1, slot) if g + 1 < NG else None
            if g < NG:
                ps[g] = sm_stage(sts)
            if g >= 1:
                pv_stage(g - 1, slot, ps[g - 1])
            sts = nxt

    x_copy(0).start()
    for cp in chunk_copies(0, 0, 0):
        cp.start()
    x_copy(1).start()

    for blk in range(2):
        x_copy(blk).wait()

        def step(c, carry, blk=blk):
            slot = c % 2
            nslot = 1 - slot

            @pl.when(c + 1 < NC)
            def _():
                for cp in chunk_copies(blk, c + 1, nslot):
                    cp.start()
            if blk == 0:
                @pl.when(c + 1 == NC)
                def _():
                    for cp in chunk_copies(1, 0, nslot):
                        cp.start()

            cur = chunk_copies(blk, c, slot)
            cur[0].wait()
            q_s[...] = jnp.dot(x_buf[blk], wq_buf[slot], preferred_element_type=F32).astype(BF16)
            cur[1].wait()
            cur[2].wait()

            attention(slot)

            cur[3].wait()

            @pl.when(c == 0)
            def _():
                acc[...] = jnp.dot(o_s[...], wo_buf[slot], preferred_element_type=F32)

            @pl.when(c > 0)
            def _():
                acc[...] += jnp.dot(o_s[...], wo_buf[slot], preferred_element_type=F32)
            return carry

        lax.fori_loop(0, NC, step, 0)
        stage[blk] = acc[...].astype(BF16)
        out_copy(blk).start()
    out_copy(0).wait()
    out_copy(1).wait()


@jax.jit
def pallas_concat_heads__mha_block_cached__mha_block_cached__near_ridge_kernel(
    A_x, A_k_cache, A_v_cache, A_wq, A_wo, B_x, B_k_cache, B_v_cache, B_wq, B_wo):
    any_spec = pl.BlockSpec(memory_space=pl.ANY)
    out = pl.pallas_call(
        _kernel,
        out_shape=jax.ShapeDtypeStruct((M, 2 * D), BF16),
        in_specs=[any_spec] * 10,
        out_specs=any_spec,
        scratch_shapes=[
            pltpu.VMEM((2, M, D), BF16),
            pltpu.VMEM((2, D, CW), BF16),
            pltpu.VMEM((2, CW, D), BF16),
            pltpu.VMEM((2, B, HC, SK, DH), BF16),
            pltpu.VMEM((2, B, HC, SK, DH), BF16),
            pltpu.VMEM((M, CW), BF16),
            pltpu.VMEM((M, CW), BF16),
            pltpu.VMEM((M, D), F32),
            pltpu.VMEM((2, M, D), BF16),
            pltpu.SemaphoreType.DMA((2,)),
            pltpu.SemaphoreType.DMA((4, 2)),
            pltpu.SemaphoreType.DMA((2,)),
        ],
        compiler_params=pltpu.CompilerParams(vmem_limit_bytes=64 * 1024 * 1024),
    )(A_x.reshape(M, D), A_k_cache, A_v_cache, A_wq, A_wo,
      B_x.reshape(M, D), B_k_cache, B_v_cache, B_wq, B_wo)
    return out.reshape(B, SQ, 2 * D)
```

```python
import jax
import jax.numpy as jnp
from jax import lax
import jax.experimental.pallas as pl
import jax.experimental.pallas.tpu as pltpu

B, SQ, D = 32, 32, 640
H, SK, DH = 32, 32, 128
M = B * SQ
HC = 4
NC = H // HC
NS = 2 * NC
CW = HC * DH
NG = B // 4
XC = 4
XR = M // XC
SCALE = DH ** -0.5
F32 = jnp.float32
BF16 = jnp.bfloat16


def _kernel(ax, ak, av, awq, awo, bx, bk, bv, bwq, bwo, out_hbm,
            x_buf, wq_buf, wo_buf, k_buf, v_buf, q_s, o_s, acc, stage,
            sem_x, sem_w, sem_o):
    blocks = ((ax, ak, av, awq, awo), (bx, bk, bv, bwq, bwo))

    def wq_copy(blk, c, slot):
        return pltpu.make_async_copy(blocks[blk][3].at[:, pl.ds(c * CW, CW)], wq_buf.at[slot], sem_w.at[0, slot])

    def kvo_copies(blk, c, slot):
        _, k, v, _, wo = blocks[blk]
        return (
            pltpu.make_async_copy(k.at[:, pl.ds(c * HC, HC)], k_buf.at[slot], sem_w.at[1, slot]),
            pltpu.make_async_copy(v.at[:, pl.ds(c * HC, HC)], v_buf.at[slot], sem_w.at[2, slot]),
            pltpu.make_async_copy(wo.at[pl.ds(c * CW, CW), :], wo_buf.at[slot], sem_w.at[3, slot]),
        )

    def xa_copy(j):
        return pltpu.make_async_copy(ax.at[pl.ds(j * XR, XR), :], x_buf.at[0, pl.ds(j * XR, XR), :], sem_x.at[j])

    def xb_copy():
        return pltpu.make_async_copy(bx, x_buf.at[1], sem_x.at[XC])

    def outa_copy():
        return pltpu.make_async_copy(stage.at[0], out_hbm.at[:, pl.ds(0, D)], sem_o.at[XC])

    def outb_copy(j):
        return pltpu.make_async_copy(stage.at[1, pl.ds(j * XR, XR), :],
                                     out_hbm.at[pl.ds(j * XR, XR), pl.ds(D, D)], sem_o.at[j])

    def when(cond):
        if isinstance(cond, bool):
            return (lambda f: f()) if cond else (lambda f: None)
        return pl.when(cond)

    def in_range(s, lo, hi):
        if isinstance(s, int):
            return lo <= s < hi
        return jnp.logical_and(s >= lo, s < hi)

    def start_for_step(s_w, s_kvo, slot_w, slot_kvo):
        for blk in range(2):
            lo, hi = blk * NC, (blk + 1) * NC

            @when(in_range(s_kvo, lo, hi))
            def _():
                for cp in kvo_copies(blk, s_kvo - lo, slot_kvo):
                    cp.start()

            @when(in_range(s_w, lo, hi))
            def _():
                wq_copy(blk, s_w - lo, slot_w).start()

    lane_blk = lax.broadcasted_iota(jnp.int32, (SQ, 128), 1) // SQ

    def st_stage(g, slot):
        r0 = g * 128
        b0 = g * 4
        sts = []
        for h in range(HC):
            q4 = q_s[pl.ds(r0, 128), h * DH:(h + 1) * DH]
            k4 = k_buf[slot, pl.ds(b0, 4), h].reshape(128, DH)
            sts.append(lax.dot_general(k4, q4, (((1,), (1,)), ((), ())), preferred_element_type=F32))
        return sts

    def sm_stage(sts):
        pts = []
        for st in sts:
            t = st[0:SK]
            for j in range(1, 4):
                t = jnp.where(lane_blk == j, st[SK * j:SK * (j + 1)], t)
            m = jnp.max(t, axis=0, keepdims=True)
            e = jnp.exp((t - m) * SCALE)
            l = jnp.sum(e, axis=0, keepdims=True)
            pts.append(e * (1.0 / l))
        pt_all = jnp.concatenate(pts, axis=0)
        return pt_all.T

    def pv_stage(g, slot, p_all):
        r0 = g * 128
        b0 = g * 4
        for b in range(4):
            pb = p_all[SQ * b:SQ * (b + 1)]
            p_bd = jnp.concatenate(
                [jnp.where(lane_blk == h, pb, 0.0) for h in range(HC)], axis=0).astype(BF16)
            v4 = v_buf[slot, b0 + b].reshape(128, DH)
            ob = jnp.dot(p_bd, v4, preferred_element_type=F32)
            for h in range(HC):
                o_s[pl.ds(r0 + SQ * b, SQ), h * DH:(h + 1) * DH] = ob[SQ * h:SQ * (h + 1)].astype(BF16)

    def qproj_rows(xblk, slot, r0, nrows):
        q_s[pl.ds(r0, nrows), :] = jnp.dot(
            x_buf[xblk, pl.ds(r0, nrows), :], wq_buf[slot], preferred_element_type=F32).astype(BF16)

    def attention(slot, hook):
        ps = [None] * NG
        sts = st_stage(0, slot)
        for g in range(NG + 1):
            nxt = st_stage(g + 1, slot) if g + 1 < NG else None
            hook(g)
            if g < NG:
                ps[g] = sm_stage(sts)
            if g >= 1:
                pv_stage(g - 1, slot, ps[g - 1])
            sts = nxt

    def body(s, slot, last):
        c = s % NC
        if not last:
            start_for_step(s + 2, s + 1, slot, 1 - slot)

            @when(s + 1 == NC)
            def _():
                xb_copy().wait()
            wq_copy(0, 0, 1 - slot).wait()
        kvo = kvo_copies(0, 0, slot)
        kvo[0].wait()
        kvo[1].wait()
        xblk = (s + 1) // NC

        def hook(g):
            if not last and g < NG:
                qproj_rows(xblk, 1 - slot, g * 128, 128)
        attention(slot, hook)
        kvo[2].wait()
        if last:
            for j in range(XC):
                rows = pl.ds(j * XR, XR)
                stage[1, rows, :] = (acc[rows, :] + jnp.dot(
                    o_s[rows, :], wo_buf[slot], preferred_element_type=F32)).astype(BF16)
                outb_copy(j).start()
        else:
            prev = jnp.where(c == 0, 0.0, acc[...])
            acc[...] = prev + jnp.dot(o_s[...], wo_buf[slot], preferred_element_type=F32)

            @when(s == NC - 1)
            def _():
                stage[0] = acc[...].astype(BF16)
                outa_copy().start()

    wq_copy(0, 0, 0).start()
    for j in range(XC):
        xa_copy(j).start()
    wq_copy(0, 0, 0).wait()
    for j in range(XC):
        xa_copy(j).wait()
        if j == 0:
            kvo0 = kvo_copies(0, 0, 0)
            kvo0[0].start()
            kvo0[1].start()
            wq_copy(0, 1, 1).start()
            kvo0[2].start()
            xb_copy().start()
        qproj_rows(0, 0, j * XR, XR)

    def loop_body(s, carry):
        body(s, s % 2, False)
        return carry
    lax.fori_loop(0, NS - 1, loop_body, 0)
    body(NS - 1, 1, True)
    outa_copy().wait()
    for j in range(XC):
        outb_copy(j).wait()


@jax.jit
def pallas_concat_heads__mha_block_cached__mha_block_cached__near_ridge_kernel(
    A_x, A_k_cache, A_v_cache, A_wq, A_wo, B_x, B_k_cache, B_v_cache, B_wq, B_wo):
    any_spec = pl.BlockSpec(memory_space=pl.ANY)
    out = pl.pallas_call(
        _kernel,
        out_shape=jax.ShapeDtypeStruct((M, 2 * D), BF16),
        in_specs=[any_spec] * 10,
        out_specs=any_spec,
        scratch_shapes=[
            pltpu.VMEM((2, M, D), BF16),
            pltpu.VMEM((2, D, CW), BF16),
            pltpu.VMEM((2, CW, D), BF16),
            pltpu.VMEM((2, B, HC, SK, DH), BF16),
            pltpu.VMEM((2, B, HC, SK, DH), BF16),
            pltpu.VMEM((M, CW), BF16),
            pltpu.VMEM((M, CW), BF16),
            pltpu.VMEM((M, D), F32),
            pltpu.VMEM((2, M, D), BF16),
            pltpu.SemaphoreType.DMA((XC + 1,)),
            pltpu.SemaphoreType.DMA((4, 2)),
            pltpu.SemaphoreType.DMA((XC + 1,)),
        ],
        compiler_params=pltpu.CompilerParams(vmem_limit_bytes=64 * 1024 * 1024, disable_bounds_checks=True),
    )(A_x.reshape(M, D), A_k_cache, A_v_cache, A_wq, A_wo,
      B_x.reshape(M, D), B_k_cache, B_v_cache, B_wq, B_wo)
    return out.reshape(B, SQ, 2 * D)
```

```python
import jax
import jax.numpy as jnp
from jax import lax
import jax.experimental.pallas as pl
import jax.experimental.pallas.tpu as pltpu

B, SQ, D = 32, 32, 640
H, SK, DH = 32, 32, 128
M = B * SQ
HC = 4
NC = H // HC
NS = 2 * NC
CW = HC * DH
NG = B // 4
XC = 4
XR = M // XC
OUT_CHUNKS = ((0, 256), (256, 256), (512, 256), (768, 128), (896, 128))
OUT_HOOKS = {3: 0, 5: 1, 7: 2, 8: 3}
SCALE = DH ** -0.5
F32 = jnp.float32
BF16 = jnp.bfloat16


def _kernel(ax, ak, av, awq, awo, bx, bk, bv, bwq, bwo, out_hbm,
            x_buf, wq_buf, wo_buf, k_buf, v_buf, q_s, o_s, acc, stage,
            sem_x, sem_w, sem_o):
    blocks = ((ax, ak, av, awq, awo), (bx, bk, bv, bwq, bwo))

    def wq_copy(blk, c, slot):
        return pltpu.make_async_copy(
            blocks[blk][3].at[:, pl.ds(c * CW, CW)], wq_buf.at[slot], sem_w.at[0, slot])

    def kvo_copies(blk, c, slot):
        _, k, v, _, wo = blocks[blk]
        return (
            pltpu.make_async_copy(k.at[:, pl.ds(c * HC, HC)], k_buf.at[slot], sem_w.at[1, slot]),
            pltpu.make_async_copy(v.at[:, pl.ds(c * HC, HC)], v_buf.at[slot], sem_w.at[2, slot]),
            pltpu.make_async_copy(wo.at[pl.ds(c * CW, CW), :], wo_buf.at[slot], sem_w.at[3, slot]),
        )

    def xa_copy(j):
        return pltpu.make_async_copy(
            ax.at[pl.ds(j * XR, XR), :], x_buf.at[0, pl.ds(j * XR, XR), :], sem_x.at[j])

    def xb_copy():
        return pltpu.make_async_copy(bx, x_buf.at[1], sem_x.at[XC])

    def outa_copy():
        return pltpu.make_async_copy(
            stage.at[0], out_hbm.at[:, pl.ds(0, D)], sem_o.at[len(OUT_CHUNKS)])

    def outb_copy(j):
        r0, nr = OUT_CHUNKS[j]
        return pltpu.make_async_copy(
            stage.at[1, pl.ds(r0, nr), :], out_hbm.at[pl.ds(r0, nr), pl.ds(D, D)], sem_o.at[j])

    def start_prefetch(s_w, s_kvo, slot_w, slot_kvo):
        for blk in range(2):
            lo, hi = blk * NC, (blk + 1) * NC

            @pl.when(jnp.logical_and(s_kvo >= lo, s_kvo < hi))
            def _():
                for cp in kvo_copies(blk, s_kvo - lo, slot_kvo):
                    cp.start()

            @pl.when(jnp.logical_and(s_w >= lo, s_w < hi))
            def _():
                wq_copy(blk, s_w - lo, slot_w).start()

    lane_blk = lax.broadcasted_iota(jnp.int32, (SQ, 128), 1) // SQ

    def st_stage(g, slot):
        r0, b0 = g * 128, g * 4
        sts = []
        for h in range(HC):
            q4 = q_s[pl.ds(r0, 128), h * DH:(h + 1) * DH]
            k4 = k_buf[slot, pl.ds(b0, 4), h].reshape(128, DH)
            sts.append(lax.dot_general(k4, q4, (((1,), (1,)), ((), ())),
                                       preferred_element_type=F32))
        return sts

    def sm_stage(sts):
        pts = []
        for st in sts:
            t = st[0:SK]
            for j in range(1, 4):
                t = jnp.where(lane_blk == j, st[SK * j:SK * (j + 1)], t)
            m = jnp.max(t, axis=0, keepdims=True)
            e = jnp.exp((t - m) * SCALE)
            l = jnp.sum(e, axis=0, keepdims=True)
            pts.append(e * (1.0 / l))
        pt_all = jnp.concatenate(pts, axis=0)
        return pt_all.T

    def pv_stage(g, slot, p_all):
        r0, b0 = g * 128, g * 4
        for b in range(4):
            pb = p_all[SQ * b:SQ * (b + 1)]
            p_bd = jnp.concatenate(
                [jnp.where(lane_blk == h, pb, 0.0) for h in range(HC)], axis=0).astype(BF16)
            v4 = v_buf[slot, b0 + b].reshape(128, DH)
            ob = jnp.dot(p_bd, v4, preferred_element_type=F32)
            for h in range(HC):
                o_s[pl.ds(r0 + SQ * b, SQ), h * DH:(h + 1) * DH] = (
                    ob[SQ * h:SQ * (h + 1)].astype(BF16))

    def qproj_rows(xblk, wslot, r0, nrows):
        q_s[pl.ds(r0, nrows), :] = jnp.dot(
            x_buf[xblk, pl.ds(r0, nrows), :], wq_buf[wslot],
            preferred_element_type=F32).astype(BF16)

    def attention(slot, hook):
        ps = [None] * NG
        sts = st_stage(0, slot)
        for g in range(NG + 1):
            nxt = st_stage(g + 1, slot) if g + 1 < NG else None
            hook(g)
            if g < NG:
                ps[g] = sm_stage(sts)
            if g >= 1:
                pv_stage(g - 1, slot, ps[g - 1])
            sts = nxt

    def step(s, carry):
        slot = s % 2
        start_prefetch(s + 2, s + 1, slot, 1 - slot)

        @pl.when(s + 1 == NC)
        def _():
            xb_copy().wait()
        wq_copy(0, 0, 1 - slot).wait()
        kvo = kvo_copies(0, 0, slot)
        kvo[0].wait()
        kvo[1].wait()
        xblk = (s + 1) // NC

        def hook(g):
            if g < NG:
                qproj_rows(xblk, 1 - slot, g * 128, 128)
        attention(slot, hook)
        kvo[2].wait()
        prev = jnp.where(s % NC == 0, 0.0, acc[...])
        acc[...] = prev + jnp.dot(o_s[...], wo_buf[slot], preferred_element_type=F32)

        @pl.when(s == NC - 1)
        def _():
            stage[0] = acc[...].astype(BF16)
            outa_copy().start()
        return carry

    def last_step(slot):
        for cp in kvo_copies(0, 0, slot):
            cp.wait()

        def out_chunk(j):
            rows = pl.ds(*OUT_CHUNKS[j])
            stage[1, rows, :] = (acc[rows, :] + jnp.dot(
                o_s[rows, :], wo_buf[slot], preferred_element_type=F32)).astype(BF16)
            outb_copy(j).start()

        def hook(g):
            if g in OUT_HOOKS:
                out_chunk(OUT_HOOKS[g])
        attention(slot, hook)
        out_chunk(len(OUT_CHUNKS) - 1)

    wq_copy(0, 0, 0).start()
    for j in range(XC):
        xa_copy(j).start()
    wq_copy(0, 0, 0).wait()
    for j in range(XC):
        xa_copy(j).wait()
        if j == 0:
            kvo0 = kvo_copies(0, 0, 0)
            kvo0[0].start()
            kvo0[1].start()
            wq_copy(0, 1, 1).start()
            kvo0[2].start()
            xb_copy().start()
        qproj_rows(0, 0, j * XR, XR)

    lax.fori_loop(0, NS - 1, step, 0)
    last_step((NS - 1) % 2)
    outa_copy().wait()
    for j in range(len(OUT_CHUNKS)):
        outb_copy(j).wait()


@jax.jit
def pallas_concat_heads__mha_block_cached__mha_block_cached__near_ridge_kernel(
    A_x, A_k_cache, A_v_cache, A_wq, A_wo, B_x, B_k_cache, B_v_cache, B_wq, B_wo):
    any_spec = pl.BlockSpec(memory_space=pl.ANY)
    out = pl.pallas_call(
        _kernel,
        out_shape=jax.ShapeDtypeStruct((M, 2 * D), BF16),
        in_specs=[any_spec] * 10,
        out_specs=any_spec,
        scratch_shapes=[
            pltpu.VMEM((2, M, D), BF16),
            pltpu.VMEM((2, D, CW), BF16),
            pltpu.VMEM((2, CW, D), BF16),
            pltpu.VMEM((2, B, HC, SK, DH), BF16),
            pltpu.VMEM((2, B, HC, SK, DH), BF16),
            pltpu.VMEM((M, CW), BF16),
            pltpu.VMEM((M, CW), BF16),
            pltpu.VMEM((M, D), F32),
            pltpu.VMEM((2, M, D), BF16),
            pltpu.SemaphoreType.DMA((XC + 1,)),
            pltpu.SemaphoreType.DMA((4, 2)),
            pltpu.SemaphoreType.DMA((len(OUT_CHUNKS) + 1,)),
        ],
        compiler_params=pltpu.CompilerParams(
            vmem_limit_bytes=64 * 1024 * 1024, disable_bounds_checks=True),
    )(A_x.reshape(M, D), A_k_cache, A_v_cache, A_wq, A_wo,
      B_x.reshape(M, D), B_k_cache, B_v_cache, B_wq, B_wo)
    return out.reshape(B, SQ, 2 * D)
```
